```python
import os as _os
_os.environ.setdefault('JAX_PLATFORMS', 'cpu')
import jax
import jax.numpy as jnp

def _softmax(x, axis=-1):
    return jax.nn.softmax(x, axis=axis)

def _gelu(x):
    return jax.nn.gelu(x, approximate=True)

def _silu(x):
    return jax.nn.silu(x)

def _sigmoid(x):
    return jax.nn.sigmoid(x)

def _layernorm(x, axis=-1, eps=1e-05):
    m = jnp.mean(x, axis=axis, keepdims=True)
    v = jnp.var(x, axis=axis, keepdims=True)
    return (x - m) / jnp.sqrt(v + eps)

def _scatter_add(tgt, idx, src, axis=0):
    return tgt.at[idx].add(src)

def _segment_sum(src, seg, n):
    return jax.ops.segment_sum(src, seg, n)

class _Rng:

    def __init__(self, key):
        self._k = key

    def _next(self):
        self._k, sub = jax.random.split(self._k)
        return sub

    def normal(self, shape):
        return jax.random.normal(self._next(), shape, dtype=jnp.bfloat16)

    def randint(self, lo, hi, shape):
        return jax.random.randint(self._next(), shape, lo, hi, dtype=jnp.int32)

    def uniform(self, shape, lo=0.0, hi=1.0):
        return jax.random.uniform(self._next(), shape, jnp.bfloat16, lo, hi)

    def permutation(self, n):
        return jax.random.permutation(self._next(), n)
kernel_name = 'standalone__autoregressive_conv_wavenet__speech'

def setup_inputs():
    _rng = _Rng(jax.random.key(int.from_bytes(__import__("os").urandom(4), "little")))
    _w = lambda a: (lambda t: t.astype(jnp.bfloat16) if jnp.issubdtype(t.dtype, jnp.floating) else t)(jnp.asarray(a))
    B, T, D, K = (2, 4000, 512, 31)
    return {'x': _w((lambda *s: _rng.normal(s) * 0.05)(B, T, D)), 'w': _w((lambda *s: _rng.normal(s) * 0.05)(K, D, 2 * D)), 'w_o': _w((lambda *s: _rng.normal(s) * 0.05)(D, D))}

def reference(x, w, w_o):
    B, T, D = x.shape
    K = w.shape[0]
    dil = 2
    pad = (K - 1) * dil
    xp = jnp.pad(x, ((0, 0), (pad, 0), (0, 0)))
    h = jnp.einsum('btc,cd->btd', xp[:, pad:pad + T, :], w[0])
    for i in range(1, K):
        off = pad - i * dil
        h = h + jnp.einsum('btc,cd->btd', xp[:, off:off + T, :], w[i])
    f = h[..., :D].copy()
    g = h[..., D:].copy()
    z = jnp.tanh(f) * _sigmoid(g)
    return z @ w_o
```

```python
import jax
import jax.numpy as jnp
import jax.experimental.pallas as pl
import jax.experimental.pallas.tpu as pltpu

TM = 2000
HALO = 80
DIL = 2
NPH = 8


def _kernel(x_cur_ref, x_halo_ref, w_hbm, wo_ref, o_ref, xs_ref, acc_ref, w_vmem, sems):
    b = pl.program_id(0)
    t = pl.program_id(1)
    K = w_hbm.shape[0]
    D = o_ref.shape[-1]
    first = jnp.logical_and(b == 0, t == 0)

    def w_copy(i):
        return pltpu.make_async_copy(w_hbm.at[i], w_vmem.at[i], sems.at[i])

    @pl.when(first)
    def _():
        for i in range(K):
            w_copy(i).start()

    halo = x_halo_ref[16:HALO, :]
    halo = jnp.where(t == 0, jnp.zeros_like(halo), halo)
    xs_ref[0, 0:64, :] = halo
    xs_ref[0, 64:64 + TM, :] = x_cur_ref[...]
    for p in range(1, NPH):
        xs_ref[p, 16:64 + TM, :] = xs_ref[0, pl.ds(16 - DIL * p, TM + 48), :]

    def tap(i):
        @pl.when(first)
        def _():
            w_copy(i).wait()
        p = i % NPH
        j = i // NPH
        start = pl.multiple_of(64 - j * 16, 16)
        lhs = xs_ref[p, pl.ds(start, TM), :]
        return jnp.dot(lhs, w_vmem[i], preferred_element_type=jnp.float32)

    acc_ref[...] = tap(0)

    def body(i, carry):
        part = tap(i)
        acc_ref[...] += part
        return carry

    jax.lax.fori_loop(1, K, body, 0)

    h = acc_ref[...]
    f = h[:, :D]
    g = h[:, D:]
    z = (jnp.tanh(f) * jax.nn.sigmoid(g)).astype(jnp.bfloat16)
    o_ref[...] = jnp.dot(z, wo_ref[...], preferred_element_type=jnp.float32).astype(o_ref.dtype)


@jax.jit
def pallas_standalone__autoregressive_conv_wavenet__speech_kernel(
    x: jax.Array,
    w: jax.Array,
    w_o: jax.Array,
):
    B, T, D = x.shape
    K = w.shape[0]
    assert T % TM == 0 and TM % HALO == 0 and DIL * (K - 1) <= 60 and K <= 32
    halo_per_tile = TM // HALO

    return pl.pallas_call(
        _kernel,
        grid=(B, T // TM),
        in_specs=[
            pl.BlockSpec((None, TM, D), lambda b, t: (b, t, 0)),
            pl.BlockSpec((None, HALO, D),
                         lambda b, t: (b, jnp.maximum(t * halo_per_tile - 1, 0), 0)),
            pl.BlockSpec(memory_space=pl.ANY),
            pl.BlockSpec((D, D), lambda b, t: (0, 0)),
        ],
        out_specs=pl.BlockSpec((None, TM, D), lambda b, t: (b, t, 0)),
        out_shape=jax.ShapeDtypeStruct((B, T, D), jnp.bfloat16),
        scratch_shapes=[
            pltpu.VMEM((NPH, TM + 64, D), jnp.bfloat16),
            pltpu.VMEM((TM, 2 * D), jnp.float32),
            pltpu.VMEM(w.shape, w.dtype),
            pltpu.SemaphoreType.DMA((K,)),
        ],
        compiler_params=pltpu.CompilerParams(
            dimension_semantics=("arbitrary", "arbitrary"),
            vmem_limit_bytes=100 * 1024 * 1024,
        ),
    )(x, x, w, w_o)
```

```python
import jax
import jax.numpy as jnp
import jax.experimental.pallas as pl
import jax.experimental.pallas.tpu as pltpu

TM = 2000
HALO = 80
DIL = 2
NPH = 4
G = 2
STEP = DIL * NPH


def _kernel(x_cur_ref, x_halo_ref, w_hbm, wo_ref, o_ref, xs_ref, acc_ref, w_vmem, sems):
    b = pl.program_id(0)
    t = pl.program_id(1)
    D = o_ref.shape[-1]
    K = w_hbm.shape[0] // D
    first = jnp.logical_and(b == 0, t == 0)
    n_full = K // G
    rem = K - n_full * G
    peeled = list(range(n_full * G, K)) if rem else list(range((n_full - 1) * G, K))
    n_loop = n_full if rem else n_full - 1

    def w_copy(i):
        return pltpu.make_async_copy(
            w_hbm.at[pl.ds(i * D, D)], w_vmem.at[pl.ds(i * D, D)], sems.at[i])

    @pl.when(first)
    def _():
        for i in peeled + [i for i in range(K) if i not in peeled]:
            w_copy(i).start()

    halo = x_halo_ref[16:HALO, :]
    halo = jnp.where(t == 0, jnp.zeros_like(halo), halo)
    xs_ref[0, 0:64, 0:D] = halo
    xs_ref[0, 64:64 + TM, 0:D] = x_cur_ref[...]
    for p in range(1, NPH):
        q, c = divmod(p, G)
        xs_ref[q, STEP:64 + TM, c * D:(c + 1) * D] = (
            xs_ref[0, pl.ds(STEP - DIL * p, TM + 64 - STEP), 0:D])

    def group(i0, n, static):
        @pl.when(first)
        def _():
            for d in range(n):
                w_copy(i0 + d).wait()
        q = (i0 % NPH) // G
        j = i0 // NPH
        start = 64 - j * STEP
        wrow = i0 * D
        if not static:
            start = pl.multiple_of(start, STEP)
            wrow = pl.multiple_of(wrow, D)
        lhs = xs_ref[q, pl.ds(start, TM), 0:n * D]
        rhs = w_vmem[pl.ds(wrow, n * D), :]
        return jnp.dot(lhs, rhs, preferred_element_type=jnp.float32)

    acc_ref[...] = group(peeled[0], len(peeled), True)

    def body(g, carry):
        part = group(g * G, G, False)
        acc_ref[...] += part
        return carry

    jax.lax.fori_loop(0, n_loop, body, 0)

    h = acc_ref[...]
    z = (jnp.tanh(h[:, :D]) * jax.nn.sigmoid(h[:, D:])).astype(jnp.bfloat16)
    o_ref[...] = jnp.dot(z, wo_ref[...], preferred_element_type=jnp.float32).astype(o_ref.dtype)


@jax.jit
def pallas_standalone__autoregressive_conv_wavenet__speech_kernel(
    x: jax.Array,
    w: jax.Array,
    w_o: jax.Array,
):
    B, T, D = x.shape
    K = w.shape[0]
    assert T % TM == 0 and TM % HALO == 0 and DIL * (K - 1) <= 64 - STEP + 4 and K <= 32
    halo_per_tile = TM // HALO
    w2 = w.reshape(K * D, 2 * D)

    return pl.pallas_call(
        _kernel,
        grid=(B, T // TM),
        in_specs=[
            pl.BlockSpec((None, TM, D), lambda b, t: (b, t, 0)),
            pl.BlockSpec((None, HALO, D),
                         lambda b, t: (b, jnp.maximum(t * halo_per_tile - 1, 0), 0)),
            pl.BlockSpec(memory_space=pl.ANY),
            pl.BlockSpec((D, D), lambda b, t: (0, 0)),
        ],
        out_specs=pl.BlockSpec((None, TM, D), lambda b, t: (b, t, 0)),
        out_shape=jax.ShapeDtypeStruct((B, T, D), jnp.bfloat16),
        scratch_shapes=[
            pltpu.VMEM((NPH // G, TM + 64, G * D), jnp.bfloat16),
            pltpu.VMEM((TM, 2 * D), jnp.float32),
            pltpu.VMEM(w2.shape, w.dtype),
            pltpu.SemaphoreType.DMA((K,)),
        ],
        compiler_params=pltpu.CompilerParams(
            dimension_semantics=("arbitrary", "arbitrary"),
            vmem_limit_bytes=100 * 1024 * 1024,
        ),
    )(x, x, w2, w_o)
```

```python
import jax
import jax.numpy as jnp
import jax.experimental.pallas as pl
import jax.experimental.pallas.tpu as pltpu

TM = 2000
HALO = 80
DIL = 2
NPH = 4
G = 2
KB = 128
STEP = DIL * NPH


def _kernel(x_cur_ref, x_halo_ref, w_hbm, wo_ref, o_ref, xs_ref, acc_ref, w_vmem, sems):
    b = pl.program_id(0)
    t = pl.program_id(1)
    D = o_ref.shape[-1]
    K = w_hbm.shape[0] // D
    first = jnp.logical_and(b == 0, t == 0)
    n_full = K // G
    rem = K - n_full * G
    peeled = list(range(n_full * G, K)) if rem else list(range((n_full - 1) * G, K))
    n_loop = n_full if rem else n_full - 1

    def w_copy(i):
        return pltpu.make_async_copy(
            w_hbm.at[pl.ds(i * D, D)], w_vmem.at[pl.ds(i * D, D)], sems.at[i])

    @pl.when(first)
    def _():
        for i in peeled + [i for i in range(K) if i not in peeled]:
            w_copy(i).start()

    halo = x_halo_ref[16:HALO, :]
    halo = jnp.where(t == 0, jnp.zeros_like(halo), halo)
    xs_ref[0, 0:64, 0:D] = halo
    xs_ref[0, 64:64 + TM, 0:D] = x_cur_ref[...]
    for p in range(1, NPH):
        q, c = divmod(p, G)
        xs_ref[q, STEP:64 + TM, c * D:(c + 1) * D] = (
            xs_ref[0, pl.ds(STEP - DIL * p, TM + 64 - STEP), 0:D])

    def group(i0, n, static):
        @pl.when(first)
        def _():
            for d in range(n):
                w_copy(i0 + d).wait()
        q = (i0 % NPH) // G
        j = i0 // NPH
        start = 64 - j * STEP
        wrow = i0 * D
        if not static:
            start = pl.multiple_of(start, STEP)
            wrow = pl.multiple_of(wrow, D)
        lhs = xs_ref[q, pl.ds(start, TM), 0:n * D]
        rhs = w_vmem[pl.ds(wrow, n * D), :]
        return jnp.dot(lhs, rhs, preferred_element_type=jnp.float32)

    acc_ref[...] = group(peeled[0], len(peeled), True)

    def body(g, carry):
        part = group(g * G, G, False)
        acc_ref[...] += part
        return carry

    jax.lax.fori_loop(0, n_loop, body, 0)

    out = None
    for kb in range(D // KB):
        f = acc_ref[:, kb * KB:(kb + 1) * KB]
        g = acc_ref[:, D + kb * KB:D + (kb + 1) * KB]
        z = (jnp.tanh(f) * jax.nn.sigmoid(g)).astype(jnp.bfloat16)
        part = jnp.dot(z, wo_ref[kb * KB:(kb + 1) * KB, :], preferred_element_type=jnp.float32)
        out = part if out is None else out + part
    o_ref[...] = out.astype(o_ref.dtype)


@jax.jit
def pallas_standalone__autoregressive_conv_wavenet__speech_kernel(
    x: jax.Array,
    w: jax.Array,
    w_o: jax.Array,
):
    B, T, D = x.shape
    K = w.shape[0]
    assert T % TM == 0 and TM % HALO == 0 and 64 - STEP * ((K - 1) // NPH) >= STEP and D % KB == 0
    halo_per_tile = TM // HALO
    w2 = w.reshape(K * D, 2 * D)

    return pl.pallas_call(
        _kernel,
        grid=(B, T // TM),
        in_specs=[
            pl.BlockSpec((None, TM, D), lambda b, t: (b, t, 0)),
            pl.BlockSpec((None, HALO, D),
                         lambda b, t: (b, jnp.maximum(t * halo_per_tile - 1, 0), 0)),
            pl.BlockSpec(memory_space=pl.ANY),
            pl.BlockSpec((D, D), lambda b, t: (0, 0)),
        ],
        out_specs=pl.BlockSpec((None, TM, D), lambda b, t: (b, t, 0)),
        out_shape=jax.ShapeDtypeStruct((B, T, D), jnp.bfloat16),
        scratch_shapes=[
            pltpu.VMEM((NPH // G, TM + 64, G * D), jnp.bfloat16),
            pltpu.VMEM((TM, 2 * D), jnp.float32),
            pltpu.VMEM(w2.shape, w.dtype),
            pltpu.SemaphoreType.DMA((K,)),
        ],
        compiler_params=pltpu.CompilerParams(
            dimension_semantics=("arbitrary", "arbitrary"),
            vmem_limit_bytes=100 * 1024 * 1024,
        ),
    )(x, x, w2, w_o)
```
